```python
import jax
import jax.numpy as jnp

def _softmax(x, axis=-1):
    return jax.nn.softmax(x, axis=axis)
def _gelu(x):
    return jax.nn.gelu(x, approximate=True)
def _silu(x):
    return jax.nn.silu(x)
def _sigmoid(x):
    return jax.nn.sigmoid(x)
def _layernorm(x, axis=-1, eps=1e-5):
    m = jnp.mean(x, axis=axis, keepdims=True)
    v = jnp.var(x, axis=axis, keepdims=True)
    return (x - m) / jnp.sqrt(v + eps)
def _scatter_add(tgt, idx, src, axis=0):
    return tgt.at[idx].add(src)
def _segment_sum(src, seg, n):
    return jax.ops.segment_sum(src, seg, n)
class _Rng:
    def __init__(self, key):
        self._k = key
    def _next(self):
        self._k, sub = jax.random.split(self._k)
        return sub
    def normal(self, shape):
        return jax.random.normal(self._next(), shape, dtype=jnp.bfloat16)
    def randint(self, lo, hi, shape):
        return jax.random.randint(self._next(), shape, lo, hi, dtype=jnp.int32)
    def uniform(self, shape, lo=0.0, hi=1.0):
        return jax.random.uniform(self._next(), shape, jnp.bfloat16, lo, hi)
    def permutation(self, n):
        return jax.random.permutation(self._next(), n)


kernel_name = 'standalone__depthwise_separable__vision'

def setup_inputs():
    _rng = _Rng(jax.random.key(int.from_bytes(__import__("os").urandom(4), "little")))
    _w = (lambda a: (lambda t: t.astype(jnp.bfloat16) if jnp.issubdtype(t.dtype, jnp.floating) else t)(jnp.asarray(a)))
    H = W = 384
    C = 384
    k = 1
    return {
        "x": _w((lambda *s: _rng.normal(s) * 0.05)(1, H, W, C)),
        "dw": _w((lambda *s: _rng.normal(s) * 0.05)(k, k, C)),
        "pw": _w((lambda *s: _rng.normal(s) * 0.05)(C, C)),
    }

def reference(x, dw, pw):
    B, H, W, C = x.shape
    k = dw.shape[0]
    pad = k // 2
    xp = jnp.pad(x, ((0,0),(pad,pad),(pad,pad),(0,0)))
    out = jnp.zeros_like(x)
    for i in range(k):
        for j in range(k):
            out = out + xp[:, i:i+H, j:j+W, :] * dw[i, j][None, None, None, :]
    return jnp.einsum('bhwc,cd->bhwd', out, pw)
```

```python
import jax
import jax.numpy as jnp
import jax.experimental.pallas as pl
import jax.experimental.pallas.tpu as pltpu


@jax.jit
def pallas_standalone__depthwise_separable__vision_kernel(
    x: jax.Array,
    dw: jax.Array,
    pw: jax.Array,
):
    B, H, W, C = x.shape
    assert dw.shape == (1, 1, C)
    D = pw.shape[1]
    M = B * H * W
    tm = 2048
    assert M % tm == 0

    def kernel(x_ref, dw_ref, pw_ref, o_ref):
        xs = (x_ref[...].astype(jnp.float32) * dw_ref[...].astype(jnp.float32)).astype(x_ref.dtype)
        o_ref[...] = jnp.dot(xs, pw_ref[...], preferred_element_type=jnp.float32).astype(o_ref.dtype)

    out = pl.pallas_call(
        kernel,
        grid=(M // tm,),
        in_specs=[
            pl.BlockSpec((tm, C), lambda i: (i, 0)),
            pl.BlockSpec((1, C), lambda i: (0, 0)),
            pl.BlockSpec((C, D), lambda i: (0, 0)),
        ],
        out_specs=pl.BlockSpec((tm, D), lambda i: (i, 0)),
        out_shape=jax.ShapeDtypeStruct((M, D), x.dtype),
        compiler_params=pltpu.CompilerParams(
            dimension_semantics=("arbitrary",), vmem_limit_bytes=64 * 1024 * 1024
        ),
    )(x.reshape(M, C), dw.reshape(1, C), pw)
    return out.reshape(B, H, W, D)
```

```python
import jax
import jax.numpy as jnp
from jax import lax
import jax.experimental.pallas as pl
import jax.experimental.pallas.tpu as pltpu

_SLAB = 2048
_TC = 1024
_G = 8
_T = 16
_WG = 8
_NWS = 4
_W_PER_CHUNK = 2
_SWITCH = 0.58
_LAST = 256
_FIRST = (1, 1, 2, 4)


@jax.jit
def pallas_standalone__depthwise_separable__vision_kernel(
    x: jax.Array,
    dw: jax.Array,
    pw: jax.Array,
):
    B, H, W, C = x.shape
    assert dw.shape == (1, 1, C) and pw.shape == (C, C)
    M = B * H * W
    S, TC, G, T, WG, NWS = _SLAB, _TC, _G, _T, _WG, _NWS
    assert M % (S * G) == 0 and S % TC == 0 and S % (T * WG) == 0
    NB = M // S
    GPS = S // (T * WG)
    NGRP = (NB // G) * GPS
    CPS = S // TC
    NCH = NB * CPS
    switch = int(NCH * _SWITCH)

    reads = []
    s0 = 0
    for n in _FIRST:
        reads.append((s0, n))
        s0 += n
    while s0 < NB - 1:
        n = min(G, NB - 1 - s0)
        reads.append((s0, n))
        s0 += n
    assert s0 == NB - 1
    NR = len(reads)

    n_early = (NCH - switch) * _W_PER_CHUNK
    assert NWS <= n_early <= NGRP
    for g in range(n_early):
        assert (g // GPS + 1) * G * CPS <= switch + g // _W_PER_CHUNK

    def kernel(x_hbm, dw_hbm, pw_hbm, o_hbm, buf, dw_ref, pw_ref, rsem, wsem, psem):
        def read(k):
            if k < NR:
                idx = (pl.ds(*reads[k]),)
            elif k == NR:
                idx = (NB - 1, pl.ds(0, S - _LAST))
            else:
                idx = (NB - 1, pl.ds(S - _LAST, _LAST))
            return pltpu.make_async_copy(x_hbm.at[idx], buf.at[idx], rsem.at[k])

        def write(g, row, rows):
            idx = (pl.ds((g // GPS) * G, G), pl.ds(pl.multiple_of(row, T), rows))
            return pltpu.make_async_copy(buf.at[idx], o_hbm.at[idx], wsem.at[g % NWS])

        def wait_group(g):
            write(g, (g % GPS) * (WG * T), WG * T).wait()

        def issue_group(g):
            @pl.when(g >= NWS)
            def _():
                wait_group(g - NWS)

            for q in range(WG):
                write(g, ((g % GPS) * WG + q) * T, T).start()

        dw_copy = pltpu.make_async_copy(dw_hbm, dw_ref, psem.at[0])
        pw_copy = pltpu.make_async_copy(pw_hbm, pw_ref, psem.at[1])
        dw_copy.start(priority=0)
        pw_copy.start(priority=0)
        for k in range(NR + 2):
            read(k).start(priority=1)
        dw_copy.wait()
        pw_copy.wait()

        def body(i, carry):
            for k in range(NR):
                first_chunk = reads[k][0] * CPS
                if first_chunk < switch:
                    @pl.when(i == first_chunk)
                    def _():
                        read(k).wait()

            @pl.when(i == switch)
            def _():
                for k in range(NR + 1):
                    if k == NR or reads[k][0] * CPS >= switch:
                        read(k).wait()

            @pl.when(i >= switch)
            def _():
                for q in range(_W_PER_CHUNK):
                    issue_group((i - switch) * _W_PER_CHUNK + q)

            @pl.when(i == switch)
            def _():
                read(NR + 1).wait()

            b = i // CPS
            rows = pl.ds(pl.multiple_of((i % CPS) * TC, TC), TC)
            xs = buf[b, rows, :].astype(jnp.float32) * dw_ref[...].astype(jnp.float32)
            res = jnp.dot(xs.astype(buf.dtype), pw_ref[...],
                          preferred_element_type=jnp.float32)
            buf[b, rows, :] = res.astype(buf.dtype)
            return carry

        lax.fori_loop(0, NCH, body, 0)

        def tail(g, carry):
            issue_group(g)
            return carry

        lax.fori_loop(n_early, NGRP, tail, 0)
        for g in range(NGRP - NWS, NGRP):
            wait_group(g)

    out = pl.pallas_call(
        kernel,
        in_specs=[pl.BlockSpec(memory_space=pl.ANY)] * 3,
        out_specs=pl.BlockSpec(memory_space=pl.ANY),
        out_shape=jax.ShapeDtypeStruct((NB, S, C), x.dtype),
        scratch_shapes=[
            pltpu.VMEM((NB, S, C), x.dtype),
            pltpu.VMEM((1, C), dw.dtype),
            pltpu.VMEM((C, C), pw.dtype),
            pltpu.SemaphoreType.DMA((NR + 2,)),
            pltpu.SemaphoreType.DMA((NWS,)),
            pltpu.SemaphoreType.DMA((2,)),
        ],
        compiler_params=pltpu.CompilerParams(vmem_limit_bytes=124 * 1024 * 1024),
    )(x.reshape(NB, S, C), dw.reshape(1, C), pw)
    return out.reshape(B, H, W, C)
```

```python
import jax
import jax.numpy as jnp
from jax import lax
import jax.experimental.pallas as pl
import jax.experimental.pallas.tpu as pltpu

_S = 2048
_LANES = 128
_G1 = 24
_PR = 64
_T1 = 32
_NBA = 2
_AHEAD = 8
_RING = 16
_LAST = 24
_G0 = 4
_T0 = 8
_EVERY = 2
_N1 = 57
_G = 6
_T = 16
_K = 33
_Q = 32


def _log2(v):
    s = v.bit_length() - 1
    assert 1 << s == v
    return s


def _divmod(n, d):
    if isinstance(n, int):
        return n // d, n % d
    return lax.shift_right_logical(n, _log2(d)), n & (d - 1)


def _aligned(v, m):
    return v if isinstance(v, int) else pl.multiple_of(v, m)


@jax.jit
def pallas_standalone__depthwise_separable__vision_kernel(
    x: jax.Array,
    dw: jax.Array,
    pw: jax.Array,
):
    B, H, W, C = x.shape
    assert dw.shape == (1, 1, C) and pw.shape == (C, C)
    M = B * H * W
    S, G1, PR, G0, T0, G, T, K, Q, N1 = _S, _G1, _PR, _G0, _T0, _G, _T, _K, _Q, _N1
    TC = G1 * PR
    assert M % S == 0 and M % TC == 0
    NB = M // S
    NCH = M // TC
    CPB = S // PR
    NCA = _NBA * CPB
    NA = _NBA * G1
    NB0 = NB - NA
    J0 = S // T0
    N0 = (NB0 // G0) * J0
    NS = 2 * (G1 // _EVERY) + 3
    J = S // T
    NW = (NB // G) * J
    assert NB0 % G0 == 0 and NB % G == 0 and PR % _T1 == 0 and G1 % 4 == 0
    assert NCA - 1 - _AHEAD < N1 < NCA and _AHEAD <= _RING
    assert (N1 - 1) * NS < N0 <= N1 * NS

    def chunks_needed(group):
        last = group * G + G - 1
        if last < NA:
            return (last // G1 + 1) * CPB
        return NCA + pl.cdiv((last + 1 - NA) * S, TC)

    n_early = (NCH - N1) * K
    assert Q <= n_early <= NW
    assert all(chunks_needed(n // J) <= N1 + n // K for n in range(n_early))

    def kernel(x_hbm, dw_hbm, pw_hbm, o_hbm, buf, dw_ref, pw_ref,
               a_sem, last_sem, b_sem, w_sem, p_sem):
        def fetch(idx, sem):
            return pltpu.make_async_copy(x_hbm.at[idx], buf.at[idx], sem)

        def a_copy(c, off, rows, sem=None):
            batch, pos = _divmod(c, CPB)
            if sem is None:
                sem = a_sem.at[_divmod(c, _RING)[1]]
            return fetch((pl.ds(batch * G1, G1),
                          pl.ds(_aligned(pos * PR + off, 8), rows)), sem)

        def a_start(c):
            for off in range(0, PR, _T1):
                a_copy(c, off, _T1).start(priority=1)

        def a_start_last():
            for off in range(0, PR - _LAST, _T1):
                rows = min(_T1, PR - _LAST - off)
                a_copy(NCA - 1, off, rows, last_sem.at[0]).start(priority=1)
            a_copy(NCA - 1, PR - _LAST, _LAST, last_sem.at[1]).start(priority=1)

        def b_copy(n):
            group, j = _divmod(n, J0)
            return fetch((pl.ds(NA + group * G0, G0),
                          pl.ds(_aligned(j * T0, T0), T0)), b_sem)

        def out_copy(n):
            group, j = _divmod(n, J)
            idx = (pl.ds(group * G, G), pl.ds(_aligned(j * T, T), T))
            return pltpu.make_async_copy(buf.at[idx], o_hbm.at[idx],
                                         w_sem.at[_divmod(n, Q)[1]])

        def conv(xv):
            xs = xv.astype(jnp.float32) * dw_ref[...].astype(jnp.float32)
            res = jnp.dot(xs.astype(xv.dtype), pw_ref[...],
                          preferred_element_type=jnp.float32)
            return res.astype(xv.dtype)

        dw_copy = pltpu.make_async_copy(dw_hbm, dw_ref, p_sem.at[0])
        pw_copy = pltpu.make_async_copy(pw_hbm, pw_ref, p_sem.at[1])
        dw_copy.start(priority=0)
        pw_copy.start(priority=0)
        for c in range(_AHEAD):
            a_start(c)
        dw_copy.wait()
        pw_copy.wait()

        def phase1(i, carry):
            a_copy(i, 0, PR).wait()

            @pl.when(i + _AHEAD < NCA - 1)
            def _():
                a_start(i + _AHEAD)

            @pl.when(i + _AHEAD == NCA - 1)
            def _():
                a_start_last()

            slots = iter(range(NS))

            def b_start():
                slot = next(slots)
                n = i * NS + slot
                if (N1 - 1) * NS + slot < N0:
                    b_copy(n).start(priority=0)
                else:
                    @pl.when(n < N0)
                    def _():
                        b_copy(n).start(priority=0)

            batch, pos = _divmod(i, CPB)
            s0 = batch * G1

            def rows(off):
                return pl.ds(pl.multiple_of(pos * PR + off, 16), PR - off)

            b_start()
            head = [buf[s0 + g, rows(0), :_LANES] for g in range(G1)]
            rest = []
            for g in range(G1):
                if g % _EVERY == 0:
                    b_start()
                rest.append(buf[s0 + g, rows(0), _LANES:])
            res = conv(jnp.concatenate(
                [jnp.concatenate(head, axis=0), jnp.concatenate(rest, axis=0)], axis=1))
            for g in range(G1):
                off = 0
                if g % _EVERY == 0:
                    b_start()
                if g == 0:
                    off = 16
                    buf[s0, pl.ds(pl.multiple_of(pos * PR, 16), off), :] = res[:off]
                    b_start()
                buf[s0 + g, rows(off), :] = res[g * PR + off:(g + 1) * PR]
            b_start()
            assert next(slots, None) is None
            return carry

        lax.fori_loop(0, N1, phase1, 0)

        fetch((pl.ds(NA, NB0),), b_sem).wait()
        for c in range(N1, NCA - 1):
            a_copy(c, 0, PR).wait()
        a_copy(NCA - 1, 0, PR - _LAST, last_sem.at[0]).wait()

        def phase2(i, carry):
            for q in range(K):
                n = (i - N1) * K + q

                @pl.when(n >= Q)
                def _():
                    out_copy(n - Q).wait()

                out_copy(n).start()

            @pl.when(i == NCA - 1)
            def _():
                a_copy(NCA - 1, PR - _LAST, _LAST, last_sem.at[1]).wait()

            batch, pos = _divmod(i, CPB)
            in_a = i < NCA
            base = jnp.where(in_a, batch * (G1 * S) + pos * PR, i * TC)
            step = jnp.where(in_a, S, PR)
            pieces = []
            for g in range(G1):
                slab, row = _divmod(base + g * step, S)
                pieces.append((slab, pl.ds(pl.multiple_of(row, PR), PR)))
            res = conv(jnp.concatenate([buf[s, r, :] for s, r in pieces], axis=0))
            for g, (s, r) in enumerate(pieces):
                buf[s, r, :] = res[g * PR:(g + 1) * PR]
            return carry

        lax.fori_loop(N1, NCH, phase2, 0)

        def drain(n, carry):
            out_copy(n - Q).wait()
            out_copy(n).start()
            return carry

        lax.fori_loop(n_early, NW, drain, 0)
        for n in range(NW - Q, NW):
            out_copy(n).wait()

    out = pl.pallas_call(
        kernel,
        in_specs=[pl.BlockSpec(memory_space=pl.ANY)] * 3,
        out_specs=pl.BlockSpec(memory_space=pl.ANY),
        out_shape=jax.ShapeDtypeStruct((NB, S, C), x.dtype),
        scratch_shapes=[
            pltpu.VMEM((NB, S, C), x.dtype),
            pltpu.VMEM((1, C), dw.dtype),
            pltpu.VMEM((C, C), pw.dtype),
            pltpu.SemaphoreType.DMA((_RING,)),
            pltpu.SemaphoreType.DMA((2,)),
            pltpu.SemaphoreType.DMA,
            pltpu.SemaphoreType.DMA((Q,)),
            pltpu.SemaphoreType.DMA((2,)),
        ],
        compiler_params=pltpu.CompilerParams(
            vmem_limit_bytes=124 * 1024 * 1024,
            disable_bounds_checks=True,
            disable_semaphore_checks=True,
        ),
    )(x.reshape(NB, S, C), dw.reshape(1, C), pw)
    return out.reshape(B, H, W, C)
```

```python
import jax
import jax.numpy as jnp
from jax import lax
import jax.experimental.pallas as pl
import jax.experimental.pallas.tpu as pltpu

_S = 2048
_LANES = 128
_G1 = 24
_PR = 64
_T1 = 32
_NBA = 2
_AHEAD = 8
_RING = 16
_LAST = 24
_G0 = 4
_T0 = 8
_EVERY = 2
_N1 = 57
_G = 6
_T = 16
_K = 33
_Q = 32


def _log2(v):
    s = v.bit_length() - 1
    assert 1 << s == v
    return s


def _divmod(n, d):
    if isinstance(n, int):
        return n // d, n % d
    return lax.shift_right_logical(n, _log2(d)), n & (d - 1)


def _aligned(v, m):
    return v if isinstance(v, int) else pl.multiple_of(v, m)


def _compiler_params():
    kwargs = dict(vmem_limit_bytes=124 * 1024 * 1024, disable_bounds_checks=True)
    try:
        return pltpu.CompilerParams(disable_semaphore_checks=True, **kwargs)
    except TypeError:
        return pltpu.CompilerParams(**kwargs)


@jax.jit
def pallas_standalone__depthwise_separable__vision_kernel(
    x: jax.Array,
    dw: jax.Array,
    pw: jax.Array,
):
    B, H, W, C = x.shape
    assert dw.shape == (1, 1, C) and pw.shape == (C, C)
    M = B * H * W
    S, G1, PR, G0, T0, G, T, K, Q, N1 = _S, _G1, _PR, _G0, _T0, _G, _T, _K, _Q, _N1
    TC = G1 * PR
    assert M % S == 0 and M % TC == 0
    NB = M // S
    NCH = M // TC
    CPB = S // PR
    NCA = _NBA * CPB
    NA = _NBA * G1
    NB0 = NB - NA
    J0 = S // T0
    N0 = (NB0 // G0) * J0
    NS = 2 * (G1 // _EVERY) + 3
    J = S // T
    NW = (NB // G) * J
    assert NB0 % G0 == 0 and NB % G == 0 and PR % _T1 == 0 and G1 % 4 == 0
    assert NCA - 1 - _AHEAD < N1 < NCA and _AHEAD <= _RING
    assert (N1 - 1) * NS < N0 <= N1 * NS

    def chunks_needed(group):
        last = group * G + G - 1
        if last < NA:
            return (last // G1 + 1) * CPB
        return NCA + pl.cdiv((last + 1 - NA) * S, TC)

    n_early = (NCH - N1) * K
    assert Q <= n_early <= NW
    assert all(chunks_needed(n // J) <= N1 + n // K for n in range(n_early))

    def kernel(x_hbm, dw_hbm, pw_hbm, o_hbm, buf, dw_ref, pw_ref,
               a_sem, last_sem, b_sem, w_sem, p_sem):
        def fetch(idx, sem):
            return pltpu.make_async_copy(x_hbm.at[idx], buf.at[idx], sem)

        def a_copy(c, off, rows, sem=None):
            batch, pos = _divmod(c, CPB)
            if sem is None:
                sem = a_sem.at[_divmod(c, _RING)[1]]
            return fetch((pl.ds(batch * G1, G1),
                          pl.ds(_aligned(pos * PR + off, 8), rows)), sem)

        def a_start(c):
            for off in range(0, PR, _T1):
                a_copy(c, off, _T1).start(priority=1)

        def a_start_last():
            for off in range(0, PR - _LAST, _T1):
                rows = min(_T1, PR - _LAST - off)
                a_copy(NCA - 1, off, rows, last_sem.at[0]).start(priority=1)
            a_copy(NCA - 1, PR - _LAST, _LAST, last_sem.at[1]).start(priority=1)

        def b_copy(n):
            group, j = _divmod(n, J0)
            return fetch((pl.ds(NA + group * G0, G0),
                          pl.ds(_aligned(j * T0, T0), T0)), b_sem)

        def out_copy(n):
            group, j = _divmod(n, J)
            idx = (pl.ds(group * G, G), pl.ds(_aligned(j * T, T), T))
            return pltpu.make_async_copy(buf.at[idx], o_hbm.at[idx],
                                         w_sem.at[_divmod(n, Q)[1]])

        def conv(xv):
            xs = xv.astype(jnp.float32) * dw_ref[...].astype(jnp.float32)
            res = jnp.dot(xs.astype(xv.dtype), pw_ref[...],
                          preferred_element_type=jnp.float32)
            return res.astype(xv.dtype)

        dw_copy = pltpu.make_async_copy(dw_hbm, dw_ref, p_sem.at[0])
        pw_copy = pltpu.make_async_copy(pw_hbm, pw_ref, p_sem.at[1])
        dw_copy.start(priority=0)
        pw_copy.start(priority=0)
        for c in range(_AHEAD):
            a_start(c)
        dw_copy.wait()
        pw_copy.wait()

        def phase1(i, carry):
            a_copy(i, 0, PR).wait()

            @pl.when(i + _AHEAD < NCA - 1)
            def _():
                a_start(i + _AHEAD)

            @pl.when(i + _AHEAD == NCA - 1)
            def _():
                a_start_last()

            slots = iter(range(NS))

            def b_start():
                slot = next(slots)
                n = i * NS + slot
                if (N1 - 1) * NS + slot < N0:
                    b_copy(n).start(priority=0)
                else:
                    @pl.when(n < N0)
                    def _():
                        b_copy(n).start(priority=0)

            batch, pos = _divmod(i, CPB)
            s0 = batch * G1

            def rows(off):
                return pl.ds(pl.multiple_of(pos * PR + off, 16), PR - off)

            b_start()
            head = [buf[s0 + g, rows(0), :_LANES] for g in range(G1)]
            rest = []
            for g in range(G1):
                if g % _EVERY == 0:
                    b_start()
                rest.append(buf[s0 + g, rows(0), _LANES:])
            res = conv(jnp.concatenate(
                [jnp.concatenate(head, axis=0), jnp.concatenate(rest, axis=0)], axis=1))
            for g in range(G1):
                off = 0
                if g % _EVERY == 0:
                    b_start()
                if g == 0:
                    off = 16
                    buf[s0, pl.ds(pl.multiple_of(pos * PR, 16), off), :] = res[:off]
                    b_start()
                buf[s0 + g, rows(off), :] = res[g * PR + off:(g + 1) * PR]
            b_start()
            assert next(slots, None) is None
            return carry

        lax.fori_loop(0, N1, phase1, 0)

        fetch((pl.ds(NA, NB0),), b_sem).wait()
        for c in range(N1, NCA - 1):
            a_copy(c, 0, PR).wait()
        a_copy(NCA - 1, 0, PR - _LAST, last_sem.at[0]).wait()

        def phase2(i, carry):
            for q in range(K):
                n = (i - N1) * K + q

                @pl.when(n >= Q)
                def _():
                    out_copy(n - Q).wait()

                out_copy(n).start()

            @pl.when(i == NCA - 1)
            def _():
                a_copy(NCA - 1, PR - _LAST, _LAST, last_sem.at[1]).wait()

            batch, pos = _divmod(i, CPB)
            in_a = i < NCA
            base = jnp.where(in_a, batch * (G1 * S) + pos * PR, i * TC)
            step = jnp.where(in_a, S, PR)
            pieces = []
            for g in range(G1):
                slab, row = _divmod(base + g * step, S)
                pieces.append((slab, pl.ds(pl.multiple_of(row, PR), PR)))
            res = conv(jnp.concatenate([buf[s, r, :] for s, r in pieces], axis=0))
            for g, (s, r) in enumerate(pieces):
                buf[s, r, :] = res[g * PR:(g + 1) * PR]
            return carry

        lax.fori_loop(N1, NCH, phase2, 0)

        def drain(n, carry):
            out_copy(n - Q).wait()
            out_copy(n).start()
            return carry

        lax.fori_loop(n_early, NW, drain, 0)
        for n in range(NW - Q, NW):
            out_copy(n).wait()

    out = pl.pallas_call(
        kernel,
        in_specs=[pl.BlockSpec(memory_space=pl.ANY)] * 3,
        out_specs=pl.BlockSpec(memory_space=pl.ANY),
        out_shape=jax.ShapeDtypeStruct((NB, S, C), x.dtype),
        scratch_shapes=[
            pltpu.VMEM((NB, S, C), x.dtype),
            pltpu.VMEM((1, C), dw.dtype),
            pltpu.VMEM((C, C), pw.dtype),
            pltpu.SemaphoreType.DMA((_RING,)),
            pltpu.SemaphoreType.DMA((2,)),
            pltpu.SemaphoreType.DMA,
            pltpu.SemaphoreType.DMA((Q,)),
            pltpu.SemaphoreType.DMA((2,)),
        ],
        compiler_params=_compiler_params(),
    )(x.reshape(NB, S, C), dw.reshape(1, C), pw)
    return out.reshape(B, H, W, C)
```

```python
import jax
import jax.numpy as jnp
from jax import lax
import jax.experimental.pallas as pl
import jax.experimental.pallas.tpu as pltpu

_L = 128
_TILE = 8
_SLAB = 4096
_STEP = 64
_GP = 24
_NBA = 3
_AHEAD = 10
_RING = 64
_SPLIT = 4
_LAST = 80
_G0 = 6
_R0 = 16
_N1 = 56
_G = 6
_K = 25
_Q = 32
_ROT = 2


def _divmod(n, d):
    if isinstance(n, int):
        return n // d, n % d
    shift = d.bit_length() - 1
    assert 1 << shift == d
    return lax.shift_right_logical(n, shift), n & (d - 1)


def _rows(start, size, align):
    return pl.ds(start if isinstance(start, int) else pl.multiple_of(start, align), size)


def _compiler_params():
    kwargs = dict(vmem_limit_bytes=124 * 1024 * 1024, disable_bounds_checks=True)
    try:
        return pltpu.CompilerParams(disable_semaphore_checks=True, **kwargs)
    except TypeError:
        return pltpu.CompilerParams(**kwargs)


@jax.jit
def pallas_standalone__depthwise_separable__vision_kernel(
    x: jax.Array,
    dw: jax.Array,
    pw: jax.Array,
):
    B, H, W, C = x.shape
    assert dw.shape == (1, 1, C) and pw.shape == (C, C) and C == 3 * _L
    M = B * H * W
    L, TILE, SLAB, STEP, GP, G0, R0, G, K, Q, N1 = (
        _L, _TILE, _SLAB, _STEP, _GP, _G0, _R0, _G, _K, _Q, _N1)
    NC = C // L
    PIX = STEP
    SPS = SLAB // STEP
    NZ = M * NC // SLAB
    NCH = M // (GP * PIX)
    NA = _NBA * GP
    NU = _NBA * SPS
    NB0 = NZ - NA
    J0 = SLAB // R0
    N0 = (NB0 // G0) * J0
    NW = (NZ // G) * SPS
    assert NZ * SLAB == M * NC and NCH * GP * PIX == M
    assert NB0 % G0 == 0 and NZ % G == 0 and GP % NC == 0 and GP % _SPLIT == 0

    CPB = SPS // NC
    NCA = _NBA * CPB
    first_piece = [pl.cdiv(g * SPS, NC) for g in range(GP)]
    PPB = GP * SPS // NC
    HEAD = NC + 2
    assert NA // NC == GP

    def a_needed(c):
        return (c // CPB) * SPS + min(NC * (c % CPB) + HEAD - 1, SPS - 1)

    def a_started(c):
        return _AHEAD + NC * c + c // 2

    def pieces(i):
        if i == N1 + 1:
            return [g * SPS + CPB for g in range(GP)]
        if i > NCA:
            return [GP * i + g for g in range(GP)]
        c = i if i <= N1 else i - 1
        return [(c // CPB) * PPB + c % CPB + f for f in first_piece]

    def cuts(iters):
        out = [{t for i in iters for t in range(1, NC) if (NC * pieces(i)[g] + t) % SPS == 0}
               for g in range(GP)]
        out[0].add(1)
        return [tuple(sorted(c)) for c in out]

    n_pre = HEAD * _SPLIT
    NS = GP + 3
    n_post = N0 - n_pre - N1 * NS
    i_last = min(c for c in range(N1) if a_started(c + 1) >= NU - 2)
    n_early = (NCH - N1) * K

    assert 0 < n_post <= J0 and n_pre <= Q <= n_early <= NW and N1 + 1 < NCA
    done = {p: i for i in range(NCH) for p in pieces(i)}
    assert sorted(done) == list(range(M // PIX))
    for c in range(N1 + 1):
        for s in (NC * p + t for p in pieces(c) for t in range(NC)):
            assert (s // SPS // GP) * SPS + s % SPS <= a_needed(c) < NU - 2
    for c in range(N1):
        assert a_needed(c) < a_started(c)
        assert min(a_started(c + 1), NU) - _RING <= a_needed(c)
    for n in range(n_early):
        for slab in range(n // SPS * G, n // SPS * G + G):
            assert done[(slab * SPS + (n + _ROT) % SPS) // NC] < N1 + n // K

    def kernel(x_hbm, dw_hbm, pw_hbm, o_hbm, buf, dw_ref, pw_ref,
               a_sem, b_sem, w_sem, p_sem):
        def fetch(slab, slabs, rows, sem):
            idx = (pl.ds(slab, slabs), rows)
            return pltpu.make_async_copy(x_hbm.at[idx], buf.at[idx], sem)

        def a_copy(u):
            batch, step = _divmod(u, SPS)
            rows = _rows(step * STEP, STEP, STEP)
            if isinstance(u, int) and u == NU - 2:
                rows = pl.ds(SLAB - 2 * STEP, 2 * STEP - _LAST)
            if isinstance(u, int) and u == NU - 1:
                rows = pl.ds(SLAB - _LAST, _LAST)
            return fetch(batch * GP, GP, rows, a_sem.at[_divmod(u, _RING)[1]])

        def b_copy(n, count=1):
            group, j = _divmod(n, J0)
            return fetch(NA + group * G0, G0, _rows(j * R0, count * R0, R0), b_sem)

        def out_copy(n):
            group, step = _divmod(n, SPS)[0], _divmod(n + _ROT, SPS)[1]
            idx = (pl.ds(group * G, G), _rows(step * STEP, STEP, STEP))
            return pltpu.make_async_copy(buf.at[idx], o_hbm.at[idx],
                                         w_sem.at[_divmod(n, Q)[1]])

        def compute(locate, cuts, slot=None):
            parts = []
            for g in range(GP):
                for lo, hi in zip((0,) + cuts[g], cuts[g] + (NC,)):
                    slab, row = locate(g, lo)
                    parts.append((g if lo == 0 else None, slab,
                                  _rows(row, (hi - lo) * STEP, STEP), (NC * g + lo) * STEP))

            def load(slot, blocks):
                vals = []
                for g, slab, rows, _ in parts:
                    if g is not None and g % 2 == 0:
                        slot()
                    vals.append(buf[slab, rows, :])
                v = jnp.concatenate(vals, axis=0).astype(jnp.float32)
                v = v.reshape(GP * PIX // TILE, NC, TILE, L)
                return [v[:, c].reshape(GP * PIX, L) for c in blocks]

            if slot is None:
                slot = lambda: None
                cols = load(slot, range(NC))
            else:
                slot()
                cols = load(lambda: None, [0]) + load(slot, range(1, NC))
            xs = jnp.concatenate(cols, axis=1) * dw_ref[...].astype(jnp.float32)
            res = jnp.dot(xs.astype(buf.dtype), pw_ref[...],
                          preferred_element_type=jnp.float32)
            res = jnp.concatenate(
                [res[:, c * L:(c + 1) * L].reshape(GP * PIX // TILE, TILE, L)
                 for c in range(NC)], axis=1)
            res = res.reshape(GP * NC * STEP, L).astype(buf.dtype)
            for k, (g, slab, rows, first) in enumerate(parts):
                if k == 1 or (g is not None and g % 2 == 0):
                    slot()
                buf[slab, rows, :] = res[first:first + rows.size]
            slot()

        def batch_pos(c):
            batch = sum((c >= b * CPB).astype(jnp.int32) for b in range(1, _NBA))
            return batch, c - CPB * batch

        dw_copy = pltpu.make_async_copy(dw_hbm, dw_ref, p_sem.at[0])
        pw_copy = pltpu.make_async_copy(pw_hbm, pw_ref, p_sem.at[1])
        dw_copy.start(priority=0)
        pw_copy.start(priority=0)

        part = GP // _SPLIT
        head = [fetch((k % _SPLIT) * part, part, pl.ds(k // _SPLIT * STEP, STEP), w_sem.at[k])
                for k in range(n_pre)]
        for copy in head:
            copy.start(priority=1)
        for k, copy in enumerate(head):
            copy.wait()
            b_copy(k).start(priority=0)
            if HEAD <= k + 1 < _AHEAD:
                a_copy(k + 1).start(priority=1)
        dw_copy.wait()
        pw_copy.wait()

        def phase1(i, carry):
            batch, pos, lo, hi = carry
            for k in range(HEAD):
                @pl.when(lo + k < hi)
                def _():
                    a_copy(lo + k).wait()

            u0 = _AHEAD + NC * i + _divmod(i, 2)[0]
            u1 = jnp.minimum(u0 + NC + (i & 1), NU - 2)
            slots = iter(range(NS))

            def slot():
                k = next(slots)
                if 2 <= k <= NC + 2:
                    @pl.when(u0 + k - 2 < u1)
                    def _():
                        a_copy(u0 + k - 2).start(priority=1)
                if k == NC + 3:
                    @pl.when(i == i_last)
                    def _():
                        a_copy(NU - 2).start(priority=1)
                        a_copy(NU - 1).start(priority=1)
                b_copy(n_pre + i * NS + k).start(priority=0)

            def locate(g, t):
                row = pos * (NC * STEP) + ((NC * first_piece[g] + t) * STEP - g * SLAB)
                over, row = _divmod(row, SLAB) if t else (0, row)
                return batch * GP + g + over, row

            compute(locate, cuts(range(N1)), slot)
            assert next(slots, None) is None
            batch, pos = batch_pos(i + 1)
            return batch, pos, hi, batch * SPS + jnp.minimum(NC * pos + HEAD, SPS)

        lax.fori_loop(0, N1, phase1, tuple(jnp.int32(v) for v in (0, 0, HEAD, HEAD)))

        b_copy(N0 - n_post, n_post).start(priority=0)
        for u in range(a_needed(N1 - 1) + 1, NU - 1):
            a_copy(u).wait()

        def phase2(i, carry):
            for q in range(K):
                n = (i - N1) * K + q

                @pl.when(n >= Q)
                def _():
                    out_copy(n - Q).wait()

                out_copy(n).start()

            extra = i == N1 + 1

            @pl.when(extra)
            def _():
                a_copy(NU - 1).wait()
                fetch(NA, NB0, pl.ds(0, SLAB), b_sem).wait()

            regular = jnp.logical_and(i <= NCA, jnp.logical_not(extra))
            batch, pos = batch_pos(jnp.where(i > N1, i - 1, i))
            base = jnp.where(regular, batch * PPB + pos, jnp.where(extra, CPB, GP * i))
            step = jnp.where(extra, SPS, 1)
            rows = [(base + jnp.where(regular, first_piece[g], g * step)) * (NC * STEP)
                    for g in range(GP)]
            compute(lambda g, t: _divmod(rows[g] + t * STEP, SLAB), cuts(range(N1, NCH)))
            return carry

        lax.fori_loop(N1, NCH, phase2, 0)

        def drain(n, carry):
            out_copy(n - Q).wait()
            out_copy(n).start()
            return carry

        lax.fori_loop(n_early, NW, drain, 0)
        for n in range(NW - Q, NW):
            out_copy(n).wait()

    tiles = x.reshape(M // TILE, TILE, NC, L).transpose(0, 2, 1, 3).reshape(NZ, SLAB, L)
    out = pl.pallas_call(
        kernel,
        in_specs=[pl.BlockSpec(memory_space=pl.ANY)] * 3,
        out_specs=pl.BlockSpec(memory_space=pl.ANY),
        out_shape=jax.ShapeDtypeStruct((NZ, SLAB, L), x.dtype),
        scratch_shapes=[
            pltpu.VMEM((NZ, SLAB, L), x.dtype),
            pltpu.VMEM((1, C), dw.dtype),
            pltpu.VMEM((C, C), pw.dtype),
            pltpu.SemaphoreType.DMA((_RING,)),
            pltpu.SemaphoreType.DMA,
            pltpu.SemaphoreType.DMA((Q,)),
            pltpu.SemaphoreType.DMA((2,)),
        ],
        compiler_params=_compiler_params(),
    )(tiles, dw.reshape(1, C), pw)
    return out.reshape(M // TILE, NC, TILE, L).transpose(0, 2, 1, 3).reshape(B, H, W, C)
```

```python
import jax
import jax.numpy as jnp
from jax import lax
import jax.experimental.pallas as pl
import jax.experimental.pallas.tpu as pltpu

_L = 128
_TILE = 8
_SLAB = 4096
_STEP = 64
_GP = 24
_NBA = 3
_AHEAD = 11
_RING = 64
_SPLIT = 4
_LAST = 80
_G0 = 6
_R0 = 16
_N1 = 56
_G = 6
_K = 25
_Q = 32
_ROT = 3
_SHIFT_IN = 40
_SHIFT_OUT = 48


def _divmod(n, d):
    if isinstance(n, int):
        return n // d, n % d
    shift = d.bit_length() - 1
    assert 1 << shift == d
    return lax.shift_right_logical(n, shift), n & (d - 1)


def _rows(start, size, align):
    return pl.ds(start if isinstance(start, int) else pl.multiple_of(start, align), size)


def _compiler_params():
    kwargs = dict(vmem_limit_bytes=124 * 1024 * 1024, disable_bounds_checks=True)
    try:
        return pltpu.CompilerParams(disable_semaphore_checks=True, **kwargs)
    except TypeError:
        return pltpu.CompilerParams(**kwargs)


@jax.jit
def pallas_standalone__depthwise_separable__vision_kernel(
    x: jax.Array,
    dw: jax.Array,
    pw: jax.Array,
):
    B, H, W, C = x.shape
    assert dw.shape == (1, 1, C) and pw.shape == (C, C) and C == 3 * _L
    M = B * H * W
    L, TILE, SLAB, STEP, GP, G0, R0, G, K, Q, N1 = (
        _L, _TILE, _SLAB, _STEP, _GP, _G0, _R0, _G, _K, _Q, _N1)
    NC = C // L
    PIX = STEP
    SPS = SLAB // STEP
    NZ = M * NC // SLAB
    NCH = M // (GP * PIX)
    NA = _NBA * GP
    NU = _NBA * SPS
    NB0 = NZ - NA
    J0 = SLAB // R0
    N0 = (NB0 // G0) * J0
    NW = (NZ // G) * SPS
    assert NZ * SLAB == M * NC and NCH * GP * PIX == M
    assert NB0 % G0 == 0 and NZ % G == 0 and GP % NC == 0 and GP % _SPLIT == 0

    CPB = SPS // NC
    NCA = _NBA * CPB
    first_piece = [pl.cdiv(g * SPS, NC) for g in range(GP)]
    PPB = GP * SPS // NC
    HEAD = NC + 3
    assert NA // NC == GP

    def a_needed(c):
        return (c // CPB) * SPS + min(NC * (c % CPB) + HEAD - 1, SPS - 1)

    def a_started(c):
        return _AHEAD + NC * c + c // 2

    def pieces(i):
        if i == N1 + 1:
            return [g * SPS + CPB for g in range(GP)]
        if i > NCA:
            return [GP * i + g for g in range(GP)]
        c = i if i <= N1 else i - 1
        return [(c // CPB) * PPB + c % CPB + f for f in first_piece]

    def cuts(iters):
        out = [{t for i in iters for t in range(1, NC) if (NC * pieces(i)[g] + t) % SPS == 0}
               for g in range(GP)]
        out[0].add(1)
        return [tuple(sorted(c)) for c in out]

    n_pre = HEAD * _SPLIT
    NS = GP + 3
    i_last = min(c for c in range(N1) if a_started(c + 1) >= NU - 2)
    n_early = (NCH - N1) * K

    assert n_pre + N1 * NS == N0 and n_pre <= Q <= n_early <= NW and N1 + 1 < NCA
    assert 0 < _SHIFT_IN < STEP and 0 < _SHIFT_OUT < STEP
    done = {p: i for i in range(NCH) for p in pieces(i)}
    assert sorted(done) == list(range(M // PIX))
    for c in range(N1 + 1):
        for s in (NC * p + t for p in pieces(c) for t in range(NC)):
            assert (s // SPS // GP) * SPS + min(s % SPS + 1, SPS - 1) <= a_needed(c) < NU - 2
    for c in range(N1):
        assert a_needed(c) < a_started(c)
        assert min(a_started(c + 1), NU) - _RING <= a_needed(c)
    for n in range(n_early):
        for slab in range(n // SPS * G, n // SPS * G + G):
            for step in ((n + _ROT) % SPS, (n + _ROT - 1) % SPS):
                assert done[(slab * SPS + step) // NC] < N1 + n // K

    def kernel(x_hbm, dw_hbm, pw_hbm, o_hbm, buf, dw_ref, pw_ref,
               a_sem, b_sem, w_sem, p_sem):
        def fetch(slab, slabs, rows, sem):
            idx = (pl.ds(slab, slabs), rows)
            return pltpu.make_async_copy(x_hbm.at[idx], buf.at[idx], sem)

        def store(slab, slabs, rows, sem):
            idx = (pl.ds(slab, slabs), rows)
            return pltpu.make_async_copy(buf.at[idx], o_hbm.at[idx], sem)

        class Window:
            def __init__(self, make, slab, slabs, j, size, shift, sem):
                self.j, self.size, self.shift = j, size, shift
                self.copy = lambda rows: make(slab, slabs, rows, sem)

            def start(self, priority=0):
                j, size, shift = self.j, self.size, self.shift

                def start_main():
                    rows = _rows(j * size + (shift - size), size, TILE)
                    self.copy(rows).start(priority=priority)

                def start_edges():
                    self.copy(pl.ds(0, shift)).start(priority=priority)
                    self.copy(pl.ds(SLAB - size + shift, size - shift)).start(priority=priority)

                if isinstance(j, int):
                    (start_main if j else start_edges)()
                else:
                    pl.when(j != 0)(start_main)
                    pl.when(j == 0)(start_edges)

            def wait(self):
                self.copy(pl.ds(0, self.size)).wait()

        def a_copy(u):
            batch, j = _divmod(u, SPS)
            sem = a_sem.at[_divmod(u, _RING)[1]]
            end = SLAB - STEP + _SHIFT_IN
            if isinstance(u, int) and u == NU - 2:
                return fetch(batch * GP, GP, pl.ds(end - 2 * STEP, 2 * STEP - _LAST), sem)
            if isinstance(u, int) and u == NU - 1:
                return fetch(batch * GP, GP, pl.ds(end - _LAST, _LAST), sem)
            return Window(fetch, batch * GP, GP, j, STEP, _SHIFT_IN, sem)

        def b_start(n):
            group, j = _divmod(n, J0)
            fetch(NA + group * G0, G0, _rows(j * R0, R0, R0), b_sem).start(priority=0)

        def out_copy(n):
            group, j = _divmod(n, SPS)[0], _divmod(n + _ROT, SPS)[1]
            return Window(store, group * G, G, j, STEP, _SHIFT_OUT, w_sem.at[_divmod(n, Q)[1]])

        def compute(locate, cuts, slot=None):
            parts = []
            for g in range(GP):
                for lo, hi in zip((0,) + cuts[g], cuts[g] + (NC,)):
                    slab, row = locate(g, lo)
                    parts.append((g if lo == 0 else None, slab,
                                  _rows(row, (hi - lo) * STEP, STEP), (NC * g + lo) * STEP))

            def load(slot, blocks):
                vals = []
                for g, slab, rows, _ in parts:
                    if g is not None and g % 2 == 0:
                        slot()
                    vals.append(buf[slab, rows, :])
                v = jnp.concatenate(vals, axis=0).astype(jnp.float32)
                v = v.reshape(GP * PIX // TILE, NC, TILE, L)
                return [v[:, c].reshape(GP * PIX, L) for c in blocks]

            if slot is None:
                slot = lambda: None
                cols = load(slot, range(NC))
            else:
                slot()
                cols = load(lambda: None, [0]) + load(slot, range(1, NC))
            xs = jnp.concatenate(cols, axis=1) * dw_ref[...].astype(jnp.float32)
            res = jnp.dot(xs.astype(buf.dtype), pw_ref[...],
                          preferred_element_type=jnp.float32)
            res = jnp.concatenate(
                [res[:, c * L:(c + 1) * L].reshape(GP * PIX // TILE, TILE, L)
                 for c in range(NC)], axis=1)
            res = res.reshape(GP * NC * STEP, L).astype(buf.dtype)
            for k, (g, slab, rows, first) in enumerate(parts):
                if k == 1 or (g is not None and g % 2 == 0):
                    slot()
                buf[slab, rows, :] = res[first:first + rows.size]
            slot()

        def batch_pos(c):
            batch = sum((c >= b * CPB).astype(jnp.int32) for b in range(1, _NBA))
            return batch, c - CPB * batch

        dw_copy = pltpu.make_async_copy(dw_hbm, dw_ref, p_sem.at[0])
        pw_copy = pltpu.make_async_copy(pw_hbm, pw_ref, p_sem.at[1])
        dw_copy.start(priority=0)
        pw_copy.start(priority=0)

        part = GP // _SPLIT
        head = [Window(fetch, (k % _SPLIT) * part, part, k // _SPLIT, STEP, _SHIFT_IN, w_sem.at[k])
                for k in range(n_pre)]
        lead = n_pre // 2
        rest = head[lead:] + [a_copy(u) for u in range(HEAD, _AHEAD)]
        assert len(rest) <= n_pre
        for copy in head[:lead]:
            copy.start(priority=1)
        for k, copy in enumerate(head):
            copy.wait()
            b_start(k)
            if k < len(rest):
                rest[k].start(priority=1)
        dw_copy.wait()
        pw_copy.wait()

        def phase1(i, carry):
            batch, pos, lo, hi = carry
            for k in range(HEAD):
                @pl.when(lo + k < hi)
                def _():
                    a_copy(lo + k).wait()

            u0 = _AHEAD + NC * i + _divmod(i, 2)[0]
            u1 = jnp.minimum(u0 + NC + (i & 1), NU - 2)
            slots = iter(range(NS))

            def slot():
                k = next(slots)
                if 2 <= k <= NC + 2:
                    @pl.when(u0 + k - 2 < u1)
                    def _():
                        a_copy(u0 + k - 2).start(priority=1)
                if k == NC + 3:
                    @pl.when(i == i_last)
                    def _():
                        a_copy(NU - 2).start(priority=1)
                        a_copy(NU - 1).start(priority=1)
                b_start(n_pre + i * NS + k)

            def locate(g, t):
                row = pos * (NC * STEP) + ((NC * first_piece[g] + t) * STEP - g * SLAB)
                over, row = _divmod(row, SLAB) if t else (0, row)
                return batch * GP + g + over, row

            compute(locate, cuts(range(N1)), slot)
            assert next(slots, None) is None
            batch, pos = batch_pos(i + 1)
            return batch, pos, hi, batch * SPS + jnp.minimum(NC * pos + HEAD, SPS)

        lax.fori_loop(0, N1, phase1, tuple(jnp.int32(v) for v in (0, 0, HEAD, HEAD)))

        for u in range(a_needed(N1 - 1) + 1, NU - 1):
            a_copy(u).wait()

        def phase2(i, carry):
            for q in range(K):
                n = (i - N1) * K + q

                @pl.when(n >= Q)
                def _():
                    out_copy(n - Q).wait()

                out_copy(n).start()

            extra = i == N1 + 1

            @pl.when(extra)
            def _():
                a_copy(NU - 1).wait()
                fetch(NA, NB0, pl.ds(0, SLAB), b_sem).wait()

            regular = jnp.logical_and(i <= NCA, jnp.logical_not(extra))
            batch, pos = batch_pos(jnp.where(i > N1, i - 1, i))
            base = jnp.where(regular, batch * PPB + pos, jnp.where(extra, CPB, GP * i))
            step = jnp.where(extra, SPS, 1)
            rows = [(base + jnp.where(regular, first_piece[g], g * step)) * (NC * STEP)
                    for g in range(GP)]
            compute(lambda g, t: _divmod(rows[g] + t * STEP, SLAB), cuts(range(N1, NCH)))
            return carry

        lax.fori_loop(N1, NCH, phase2, 0)

        def drain(n, carry):
            out_copy(n - Q).wait()
            out_copy(n).start()
            return carry

        lax.fori_loop(n_early, NW, drain, 0)
        for n in range(NW - Q, NW):
            out_copy(n).wait()

    tiles = x.reshape(M // TILE, TILE, NC, L).transpose(0, 2, 1, 3).reshape(NZ, SLAB, L)
    out = pl.pallas_call(
        kernel,
        in_specs=[pl.BlockSpec(memory_space=pl.ANY)] * 3,
        out_specs=pl.BlockSpec(memory_space=pl.ANY),
        out_shape=jax.ShapeDtypeStruct((NZ, SLAB, L), x.dtype),
        scratch_shapes=[
            pltpu.VMEM((NZ, SLAB, L), x.dtype),
            pltpu.VMEM((1, C), dw.dtype),
            pltpu.VMEM((C, C), pw.dtype),
            pltpu.SemaphoreType.DMA((_RING,)),
            pltpu.SemaphoreType.DMA,
            pltpu.SemaphoreType.DMA((Q,)),
            pltpu.SemaphoreType.DMA((2,)),
        ],
        compiler_params=_compiler_params(),
    )(tiles, dw.reshape(1, C), pw)
    return out.reshape(M // TILE, NC, TILE, L).transpose(0, 2, 1, 3).reshape(B, H, W, C)
```

```python
import jax
import jax.numpy as jnp
from jax import lax
import jax.experimental.pallas as pl
import jax.experimental.pallas.tpu as pltpu

_L = 128
_TILE = 8
_SLAB = 4096
_STEP = 64
_GP = 24
_NBA = 3
_AHEAD = 11
_RING = 64
_SPLIT = 4
_G0 = 6
_R0 = 16
_N1 = 56
_G = 6
_K = 25
_Q = 32
_ROT = 3
_SHIFT_IN = 40
_SHIFT_OUT = 40


def _divmod(n, d):
    if isinstance(n, int):
        return n // d, n % d
    shift = d.bit_length() - 1
    assert 1 << shift == d
    return lax.shift_right_logical(n, shift), n & (d - 1)


def _rows(start, size, align):
    return pl.ds(start if isinstance(start, int) else pl.multiple_of(start, align), size)


def _compiler_params():
    kwargs = dict(vmem_limit_bytes=124 * 1024 * 1024, disable_bounds_checks=True)
    try:
        return pltpu.CompilerParams(disable_semaphore_checks=True, **kwargs)
    except TypeError:
        return pltpu.CompilerParams(**kwargs)


@jax.jit
def pallas_standalone__depthwise_separable__vision_kernel(
    x: jax.Array,
    dw: jax.Array,
    pw: jax.Array,
):
    B, H, W, C = x.shape
    assert dw.shape == (1, 1, C) and pw.shape == (C, C) and C == 3 * _L
    M = B * H * W
    L, TILE, SLAB, STEP, GP, G0, R0, G, K, Q, N1 = (
        _L, _TILE, _SLAB, _STEP, _GP, _G0, _R0, _G, _K, _Q, _N1)
    NC = C // L
    PIX = STEP
    SPS = SLAB // STEP
    NZ = M * NC // SLAB
    NCH = M // (GP * PIX)
    NA = _NBA * GP
    NU = _NBA * SPS
    NB0 = NZ - NA
    J0 = SLAB // R0
    N0 = (NB0 // G0) * J0
    NW = (NZ // G) * SPS
    assert NZ * SLAB == M * NC and NCH * GP * PIX == M
    assert NB0 % G0 == 0 and NZ % G == 0 and GP % NC == 0 and GP % _SPLIT == 0

    CPB = SPS // NC
    NCA = _NBA * CPB
    first_piece = [pl.cdiv(g * SPS, NC) for g in range(GP)]
    PPB = GP * SPS // NC
    HEAD = NC + 3
    assert NA // NC == GP

    def a_needed(c):
        return (c // CPB) * SPS + min(NC * (c % CPB) + HEAD - 1, SPS - 1)

    def a_started(c):
        return _AHEAD + NC * c + c // 2

    def pieces(i):
        if i == N1 + 1:
            return [g * SPS + CPB for g in range(GP)]
        if i > NCA:
            return [GP * i + g for g in range(GP)]
        c = i if i <= N1 else i - 1
        return [(c // CPB) * PPB + c % CPB + f for f in first_piece]

    def cuts(iters):
        out = [{t for i in iters for t in range(1, NC) if (NC * pieces(i)[g] + t) % SPS == 0}
               for g in range(GP)]
        out[0].add(1)
        return [tuple(sorted(c)) for c in out]

    n_pre = HEAD * _SPLIT
    NS = GP + 3
    n_early = Q + (NCH - N1) * K

    assert n_pre + N1 * NS == N0 and n_pre <= Q <= n_early <= NW and N1 + 1 < NCA
    assert a_started(N1) >= NU
    assert 0 < _SHIFT_IN < STEP and 0 < _SHIFT_OUT < STEP
    done = {p: i for i in range(NCH) for p in pieces(i)}
    assert sorted(done) == list(range(M // PIX))
    for c in range(N1 + 1):
        for s in (NC * p + t for p in pieces(c) for t in range(NC)):
            assert (s // SPS // GP) * SPS + min(s % SPS + 1, SPS - 1) <= a_needed(c) < NU - 1
    for c in range(N1):
        assert a_needed(c) < a_started(c)
        assert min(a_started(c + 1), NU) - _RING <= a_needed(c)
    for n in range(n_early):
        for slab in range(n // SPS * G, n // SPS * G + G):
            for step in ((n + _ROT) % SPS, (n + _ROT - 1) % SPS):
                assert done[(slab * SPS + step) // NC] <= N1 + max((n - Q) // K, -1)

    def kernel(x_hbm, dw_hbm, pw_hbm, o_hbm, buf, dw_ref, pw_ref,
               a_sem, b_sem, w_sem, p_sem):
        def fetch(slab, slabs, rows, sem):
            idx = (pl.ds(slab, slabs), rows)
            return pltpu.make_async_copy(x_hbm.at[idx], buf.at[idx], sem)

        def store(slab, slabs, rows, sem):
            idx = (pl.ds(slab, slabs), rows)
            return pltpu.make_async_copy(buf.at[idx], o_hbm.at[idx], sem)

        class Window:
            def __init__(self, make, slab, slabs, j, size, shift, sem):
                self.j = j
                self.main = lambda: [make(
                    slab, slabs, _rows(j * size + (shift - size), size, TILE), sem)]
                self.ends = lambda: [
                    make(slab, slabs, pl.ds(0, shift), sem),
                    make(slab, slabs, pl.ds(SLAB - size + shift, size - shift), sem)]

            def _each(self, fn, nonzero):
                def run(copies):
                    def body():
                        for copy in copies():
                            fn(copy)
                    return body

                if nonzero or isinstance(self.j, int):
                    run(self.main if nonzero or self.j else self.ends)()
                else:
                    pl.when(self.j != 0)(run(self.main))
                    pl.when(self.j == 0)(run(self.ends))

            def start(self, priority=0):
                self._each(lambda copy: copy.start(priority=priority), False)

            def wait(self, nonzero=False):
                self._each(lambda copy: copy.wait(), nonzero)

        def a_copy(u):
            batch, j = _divmod(u, SPS)
            return Window(fetch, batch * GP, GP, j, STEP, _SHIFT_IN,
                          a_sem.at[_divmod(u, _RING)[1]])

        def b_start(n):
            group, j = _divmod(n, J0)
            fetch(NA + group * G0, G0, _rows(j * R0, R0, R0), b_sem).start(priority=0)

        def out_copy(n):
            group, j = _divmod(n, SPS)[0], _divmod(n + _ROT, SPS)[1]
            return Window(store, group * G, G, j, STEP, _SHIFT_OUT, w_sem.at[_divmod(n, Q)[1]])

        def compute(locate, cuts, slot=None):
            parts = []
            for g in range(GP):
                for lo, hi in zip((0,) + cuts[g], cuts[g] + (NC,)):
                    slab, row = locate(g, lo)
                    parts.append((g if lo == 0 else None, slab,
                                  _rows(row, (hi - lo) * STEP, STEP), (NC * g + lo) * STEP))

            def load(slot, blocks):
                vals = []
                for g, slab, rows, _ in parts:
                    if g is not None and g % 2 == 0:
                        slot()
                    vals.append(buf[slab, rows, :])
                v = jnp.concatenate(vals, axis=0).astype(jnp.float32)
                v = v.reshape(GP * PIX // TILE, NC, TILE, L)
                return [v[:, c].reshape(GP * PIX, L) for c in blocks]

            if slot is None:
                slot = lambda: None
                cols = load(slot, range(NC))
            else:
                slot()
                cols = load(lambda: None, [0]) + load(slot, range(1, NC))
            xs = jnp.concatenate(cols, axis=1) * dw_ref[...].astype(jnp.float32)
            res = jnp.dot(xs.astype(buf.dtype), pw_ref[...],
                          preferred_element_type=jnp.float32)
            res = jnp.concatenate(
                [res[:, c * L:(c + 1) * L].reshape(GP * PIX // TILE, TILE, L)
                 for c in range(NC)], axis=1)
            res = res.reshape(GP * NC * STEP, L).astype(buf.dtype)
            for k, (g, slab, rows, first) in enumerate(parts):
                if k == 1 or (g is not None and g % 2 == 0):
                    slot()
                buf[slab, rows, :] = res[first:first + rows.size]
            slot()

        def batch_pos(c):
            batch = sum((c >= b * CPB).astype(jnp.int32) for b in range(1, _NBA))
            return batch, c - CPB * batch

        dw_copy = pltpu.make_async_copy(dw_hbm, dw_ref, p_sem.at[0])
        pw_copy = pltpu.make_async_copy(pw_hbm, pw_ref, p_sem.at[1])
        dw_copy.start(priority=0)
        pw_copy.start(priority=0)

        part = GP // _SPLIT
        head = [Window(fetch, (k % _SPLIT) * part, part, k // _SPLIT, STEP, _SHIFT_IN, w_sem.at[k])
                for k in range(n_pre)]
        lead = n_pre // 2
        rest = head[lead:] + [a_copy(u) for u in range(HEAD, _AHEAD)]
        assert len(rest) <= n_pre
        for copy in head[:lead]:
            copy.start(priority=1)
        for k, copy in enumerate(head):
            copy.wait()
            b_start(k)
            if k < len(rest):
                rest[k].start(priority=1)
        dw_copy.wait()
        pw_copy.wait()

        def phase1(i, carry):
            batch, pos, lo, hi = carry
            for k in range(HEAD):
                @pl.when(lo + k < hi)
                def _():
                    a_copy(lo + k).wait(nonzero=k > 0)

            u0 = _AHEAD + NC * i + _divmod(i, 2)[0]
            u1 = jnp.minimum(u0 + NC + (i & 1), NU)
            slots = iter(range(NS))

            def slot():
                k = next(slots)
                if 2 <= k <= NC + 2:
                    @pl.when(u0 + k - 2 < u1)
                    def _():
                        a_copy(u0 + k - 2).start(priority=1)
                b_start(n_pre + i * NS + k)

            def locate(g, t):
                row = pos * (NC * STEP) + ((NC * first_piece[g] + t) * STEP - g * SLAB)
                over, row = _divmod(row, SLAB) if t else (0, row)
                return batch * GP + g + over, row

            compute(locate, cuts(range(N1)), slot)
            assert next(slots, None) is None
            batch, pos = batch_pos(i + 1)
            return batch, pos, hi, batch * SPS + jnp.minimum(NC * pos + HEAD, SPS)

        lax.fori_loop(0, N1, phase1, tuple(jnp.int32(v) for v in (0, 0, HEAD, HEAD)))

        for u in range(a_needed(N1 - 1) + 1, NU - 1):
            a_copy(u).wait()

        for n in range(Q):
            out_copy(n).start()

        def drain(n, carry=None):
            out_copy(n - Q).wait()
            out_copy(n).start()
            return carry

        def phase2(i, carry):
            extra = i == N1 + 1

            @pl.when(extra)
            def _():
                a_copy(NU - 1).wait()
                fetch(NA, NB0, pl.ds(0, SLAB), b_sem).wait()

            regular = jnp.logical_and(i <= NCA, jnp.logical_not(extra))
            batch, pos = batch_pos(jnp.where(i > N1, i - 1, i))
            base = jnp.where(regular, batch * PPB + pos, jnp.where(extra, CPB, GP * i))
            step = jnp.where(extra, SPS, 1)
            rows = [(base + jnp.where(regular, first_piece[g], g * step)) * (NC * STEP)
                    for g in range(GP)]
            compute(lambda g, t: _divmod(rows[g] + t * STEP, SLAB), cuts(range(N1, NCH)))
            for q in range(K):
                drain(Q + (i - N1) * K + q)
            return carry

        lax.fori_loop(N1, NCH, phase2, 0)
        lax.fori_loop(n_early, NW, drain, 0)
        for n in range(NW - Q, NW):
            out_copy(n).wait()

    tiles = x.reshape(M // TILE, TILE, NC, L).transpose(0, 2, 1, 3).reshape(NZ, SLAB, L)
    out = pl.pallas_call(
        kernel,
        in_specs=[pl.BlockSpec(memory_space=pl.ANY)] * 3,
        out_specs=pl.BlockSpec(memory_space=pl.ANY),
        out_shape=jax.ShapeDtypeStruct((NZ, SLAB, L), x.dtype),
        scratch_shapes=[
            pltpu.VMEM((NZ, SLAB, L), x.dtype),
            pltpu.VMEM((1, C), dw.dtype),
            pltpu.VMEM((C, C), pw.dtype),
            pltpu.SemaphoreType.DMA((_RING,)),
            pltpu.SemaphoreType.DMA,
            pltpu.SemaphoreType.DMA((Q,)),
            pltpu.SemaphoreType.DMA((2,)),
        ],
        compiler_params=_compiler_params(),
    )(tiles, dw.reshape(1, C), pw)
    return out.reshape(M // TILE, NC, TILE, L).transpose(0, 2, 1, 3).reshape(B, H, W, C)
```
